```python
import jax
import jax.numpy as jnp

def _softmax(x, axis=-1):
    return jax.nn.softmax(x, axis=axis)
def _gelu(x):
    return jax.nn.gelu(x, approximate=True)
def _silu(x):
    return jax.nn.silu(x)
def _sigmoid(x):
    return jax.nn.sigmoid(x)
def _layernorm(x, axis=-1, eps=1e-5):
    m = jnp.mean(x, axis=axis, keepdims=True)
    v = jnp.var(x, axis=axis, keepdims=True)
    return (x - m) / jnp.sqrt(v + eps)
def _scatter_add(tgt, idx, src, axis=0):
    return tgt.at[idx].add(src)
def _segment_sum(src, seg, n):
    return jax.ops.segment_sum(src, seg, n)
class _Rng:
    def __init__(self, key):
        self._k = key
    def _next(self):
        self._k, sub = jax.random.split(self._k)
        return sub
    def normal(self, shape):
        return jax.random.normal(self._next(), shape, dtype=jnp.bfloat16)
    def randint(self, lo, hi, shape):
        return jax.random.randint(self._next(), shape, lo, hi, dtype=jnp.int32)
    def uniform(self, shape, lo=0.0, hi=1.0):
        return jax.random.uniform(self._next(), shape, jnp.bfloat16, lo, hi)
    def permutation(self, n):
        return jax.random.permutation(self._next(), n)


kernel_name = 'interleave_layers__sliding_local_dilated__glu_gated_geglu__prompt'

def setup_inputs():
    _rng = _Rng(jax.random.key(int.from_bytes(__import__("os").urandom(4), "little")))
    _w = (lambda a: (lambda t: t.astype(jnp.bfloat16) if jnp.issubdtype(t.dtype, jnp.floating) else t)(jnp.asarray(a)))
    def _A_setup():
        B, S, D = 1, 2048, 576
        return {
            "x": _w((lambda *s: _rng.normal(s) * 0.05)(B, S, D)),
            "wqkv": _w((lambda *s: _rng.normal(s) * 0.05)(D, 3 * D)),
            "wo": _w((lambda *s: _rng.normal(s) * 0.05)(D, D)),
        }
    _A_in = _A_setup()

    def _B_setup():
        B, S, Dm, Df = 1, 2048, 576, 4608
        return {
            "x": _w((lambda *s: _rng.normal(s) * 0.05)(B, S, Dm)),
            "w_gate": _w((lambda *s: _rng.normal(s) * 0.05)(Dm, Df) * (Dm ** -0.5)),
            "w_up": _w((lambda *s: _rng.normal(s) * 0.05)(Dm, Df) * (Dm ** -0.5)),
            "w_down": _w((lambda *s: _rng.normal(s) * 0.05)(Df, Dm) * (Df ** -0.5)),
        }
    _B_in = _B_setup()

    return {
        "A_x": _A_in["x"],
        "A_wqkv": _A_in["wqkv"],
        "A_wo": _A_in["wo"],
        "B_x": _B_in["x"],
        "B_w_gate": _B_in["w_gate"],
        "B_w_up": _B_in["w_up"],
        "B_w_down": _B_in["w_down"],
    }

def reference(A_x, A_wqkv, A_wo, B_x, B_w_gate, B_w_up, B_w_down):
    def _A_ref(x, wqkv, wo):
        B, S, D = x.shape
        H = 32; Dh = D // H
        W, dil = 8, 2
        qkv = (lambda x, *d: x.transpose(*d))((x @ wqkv).reshape(B, S, 3, H, Dh), 2, 0, 3, 1, 4)
        q, k, v = qkv[0], qkv[1], qkv[2]
        scale = Dh ** -0.5
        pos = jnp.arange(S)
        off = jnp.arange(W) * dil
        idx = pos[:, None] - off[None, :]
        mask = idx >= 0
        idx_c = jnp.where(mask, idx, 0).reshape(-1)
        kg = k[:, :, idx_c, :].reshape(B, H, S, W, Dh)
        vg = v[:, :, idx_c, :].reshape(B, H, S, W, Dh)
        logits = jnp.einsum("bhsd,bhswd->bhsw", q, kg) * scale
        logits = jnp.where(mask[None, None, :, :], logits, -1e9)
        attn = _softmax(logits, axis=-1)
        o = jnp.einsum("bhsw,bhswd->bhsd", attn, vg)
        return (lambda x, *d: x.transpose(*d))(o, 0, 2, 1, 3).reshape(B, S, D) @ wo

    def _B_ref(x, w_gate, w_up, w_down):
        g = jnp.einsum("bsd,df->bsf", x, w_gate)
        u = jnp.einsum("bsd,df->bsf", x, w_up)
        h = _gelu(g) * u
        return jnp.einsum("bsf,fd->bsd", h, w_down)

    x = A_x
    x = x + _A_ref(_layernorm(x, axis=-1), A_wqkv, A_wo)
    x = x + _B_ref(_layernorm(x, axis=-1), B_w_gate, B_w_up, B_w_down)
    x = x + _A_ref(_layernorm(x, axis=-1), A_wqkv, A_wo)
    x = x + _B_ref(_layernorm(x, axis=-1), B_w_gate, B_w_up, B_w_down)
    return x
```

```python
import functools
import jax
import jax.numpy as jnp
from jax import lax
import jax.experimental.pallas as pl
import jax.experimental.pallas.tpu as pltpu

S, D, F = 2048, 576, 4608
NH, DH, WIN, DIL = 32, 18, 8, 2
M = 512
H2, Q4 = M // 2, M // 4
NB = S // M
CF = 256
NCH = F // CF
DCH = 512
NDC = F // DCH
C0 = 0.7978845608028654
C1 = 0.044715 * C0
f32 = jnp.float32
bf16 = jnp.bfloat16


def dot(a, b):
    return jnp.dot(a, b, preferred_element_type=f32)


def dot_nt(a, b):
    return lax.dot_general(a, b, (((1,), (1,)), ((), ())), preferred_element_type=f32)


def a_ops(A11, A12, A21, A22):
    return [(A11 + A22), (A21 + A22), A11, A22, (A11 + A12), (A21 - A11), (A12 - A22)]


def b_ops(B11, B12, B21, B22):
    return [B11 + B22, B11, B12 - B22, B21 - B11, B22, B11 + B12, B21 + B22]


def c_comb(Ms):
    C11 = Ms[0] + Ms[3] - Ms[4] + Ms[6]
    C12 = Ms[2] + Ms[4]
    C21 = Ms[1] + Ms[3]
    C22 = Ms[0] - Ms[1] + Ms[2] + Ms[5]
    return C11, C12, C21, C22


def cat4(C11, C12, C21, C22):
    return jnp.concatenate([jnp.concatenate([C11, C12], axis=1),
                            jnp.concatenate([C21, C22], axis=1)], axis=0)


def layernorm_t(x):
    m = jnp.mean(x, axis=0, keepdims=True)
    d = x - m
    v = jnp.mean(d * d, axis=0, keepdims=True)
    return d * lax.rsqrt(v + 1e-5)


def kernel(x_hbm, wqkv_hbm, wo_hbm, wg_hbm, wu_hbm, wd_hbm, o_hbm,
           xin, xs, wqkv_raw, wo_raw, wg_raw, wu_raw, wd_raw,
           tmpT, wqkvT, woT, wa, wl, wd, ostage, sems, osems):
    cp_x = pltpu.make_async_copy(x_hbm, xin, sems.at[0])
    cp_qkv = pltpu.make_async_copy(wqkv_hbm, wqkv_raw, sems.at[1])
    cp_wo = pltpu.make_async_copy(wo_hbm, wo_raw, sems.at[2])
    cp_wg = pltpu.make_async_copy(wg_hbm, wg_raw, sems.at[3])
    cp_wu = pltpu.make_async_copy(wu_hbm, wu_raw, sems.at[4])
    cp_wd = pltpu.make_async_copy(wd_hbm, wd_raw, sems.at[5])
    cp_qkv.start(); cp_x.start(); cp_wo.start()
    cp_wg.start(); cp_wu.start(); cp_wd.start()

    cp_qkv.wait()
    for kg in range(5):
        kw = 128 if kg < 4 else 64
        blk = wqkv_raw[kg * 128:kg * 128 + kw, :].astype(f32)
        if kw < 128:
            blk = jnp.concatenate([blk, jnp.zeros((128 - kw, 3 * D), f32)], axis=0)
        tmpT[...] = blk.T
        for p in range(3):
            for d in range(DH):
                slab = tmpT[pl.ds(p * D + d, NH, stride=DH), :]
                r0 = p * D + d * NH
                wqkvT[r0:r0 + NH, kg * 128:(kg + 1) * 128] = slab.astype(bf16)
    cp_wo.wait()
    for ng in range(5):
        nw = 128 if ng < 4 else 64
        blk = wo_raw[:, ng * 128:ng * 128 + nw].astype(f32)
        if nw < 128:
            blk = jnp.concatenate([blk, jnp.zeros((D, 128 - nw), f32)], axis=1)
        tmpT[0:D, :] = blk
        perm = jnp.concatenate([tmpT[pl.ds(d, NH, stride=DH), :] for d in range(DH)], axis=0)
        perm = jnp.concatenate([perm, jnp.zeros((64, 128), f32)], axis=0)
        woT[ng * 128:ng * 128 + nw, :] = perm.T[0:nw, :].astype(bf16)
    cp_x.wait()
    for b in range(NB):
        xs[:, b * M:(b + 1) * M] = xin[:, b * M:(b + 1) * M].astype(f32)

    lane = lax.broadcasted_iota(jnp.int32, (NH, M), 1)

    def qkv_block(b):
        xn = layernorm_t(xs[:, b * M:(b + 1) * M]).astype(bf16)
        return dot(wqkvT[:, 0:D], xn)

    def attn_vpu(b, t, prev):
        ks = []
        logits = [None] * WIN
        for d in range(DH):
            q = t[d * NH:(d + 1) * NH, :]
            kc = t[D + d * NH:D + (d + 1) * NH, :]
            kp = prev[D + d * NH:D + (d + 1) * NH, :] if prev is not None else jnp.zeros((NH, 128), f32)
            kf = jnp.concatenate([kp, kc], axis=1)
            for w in range(WIN):
                kw_ = kc if w == 0 else pltpu.roll(kf, DIL * w, 1)[:, 128:]
                pr = q * kw_
                logits[w] = pr if logits[w] is None else logits[w] + pr
        scale = DH ** -0.5
        logits = [l * scale for l in logits]
        if b == 0:
            logits = [l if w == 0 else jnp.where(lane >= DIL * w, l, -1e9) for w, l in enumerate(logits)]
        mx = logits[0]
        for w in range(1, WIN):
            mx = jnp.maximum(mx, logits[w])
        es = [jnp.exp(l - mx) for l in logits]
        ssum = es[0]
        for w in range(1, WIN):
            ssum = ssum + es[w]
        inv = 1.0 / ssum
        ps = [e * inv for e in es]
        outs = []
        for d in range(DH):
            vc = t[2 * D + d * NH:2 * D + (d + 1) * NH, :]
            vp = prev[2 * D + d * NH:2 * D + (d + 1) * NH, :] if prev is not None else jnp.zeros((NH, 128), f32)
            vf = jnp.concatenate([vp, vc], axis=1)
            o = None
            for w in range(WIN):
                vw = vc if w == 0 else pltpu.roll(vf, DIL * w, 1)[:, 128:]
                pr = ps[w] * vw
                o = pr if o is None else o + pr
            outs.append(o)
        return jnp.concatenate(outs, axis=0).astype(bf16)

    def wo_block(b, oT):
        aT = dot(woT[:, 0:D], oT)
        xs[:, b * M:(b + 1) * M] += aT

    def attn_phase():
        cur = qkv_block(0)
        prev = None
        for b in range(NB):
            nxt = qkv_block(b + 1) if b + 1 < NB else None
            oT = attn_vpu(b, cur, prev)
            wo_block(b, oT)
            prev = cur[:, M - 128:]
            cur = nxt

    def prep_ffn():
        cp_wg.wait(); cp_wu.wait(); cp_wd.wait()

        def gu_chunk(j, _):
            c = pl.ds(pl.multiple_of(j * CF, CF), CF)
            g = wg_raw[0:512, c].astype(f32)
            u = wu_raw[0:512, c].astype(f32)
            b1 = b_ops(g[:256], u[:256], g[256:], u[256:])
            for k in range(7):
                o = b1[k]
                b2 = b_ops(o[:128, :128], o[:128, 128:], o[128:, :128], o[128:, 128:])
                for t in range(7):
                    wa[j, 7 * k + t] = b2[t].astype(bf16)
            wl[j, 0] = wg_raw[512:576, c]
            wl[j, 1] = wu_raw[512:576, c]
            return 0
        lax.fori_loop(0, NCH, gu_chunk, 0)

        def d_chunk(jd, _):
            c = pl.ds(pl.multiple_of(jd * DCH, DCH), DCH)
            wT = wd_raw[:, c].astype(f32) * 0.5
            a1 = a_ops(wT[:288, :256], wT[:288, 256:], wT[288:, :256], wT[288:, 256:])
            for k in range(7):
                o = a1[k]
                a2 = a_ops(o[:144, :128], o[:144, 128:], o[144:, :128], o[144:, 128:])
                for t in range(7):
                    wd[jd, 7 * k + t] = a2[t].astype(bf16)
            return 0
        lax.fori_loop(0, NDC, d_chunk, 0)

    def ffn_block(b, layer):
        r = pl.ds(pl.multiple_of(b * M, M), M)
        x = xs[:, r]
        xf = layernorm_t(x).T
        xl = xf[:, 512:576].astype(bf16)
        o1 = a_ops(xf[:H2, 0:256], xf[:H2, 256:512], xf[H2:, 0:256], xf[H2:, 256:512])
        ops = []
        for o in o1:
            ops += [t.astype(bf16) for t in a_ops(o[:Q4, :128], o[:Q4, 128:], o[Q4:, :128], o[Q4:, 128:])]
        accs = [None] * 49

        def stage1(j):
            Ms = []
            for k in range(7):
                m = [dot(ops[7 * k + t], wa[j, 7 * k + t]) for t in range(7)]
                Ms.append(cat4(*c_comb(m)))
            gl = dot(xl, wl[j, 0])
            ul = dot(xl, wl[j, 1])
            return Ms, gl, ul

        def act(g, u):
            z = g * (C0 + C1 * (g * g))
            a = g * u
            return a + a * jnp.tanh(z)

        def stage2(res):
            Ms, gl, ul = res
            g1, u1, g2, u2 = c_comb(Ms)
            g1 = g1 + gl[:H2]; u1 = u1 + ul[:H2]; g2 = g2 + gl[H2:]; u2 = u2 + ul[H2:]
            return act(g1, u1), act(g2, u2)

        def stage3(jd, hs):
            h1 = jnp.concatenate([h[0] for h in hs], axis=1)
            h2 = jnp.concatenate([h[1] for h in hs], axis=1)
            hc = DCH // 2
            qc = DCH // 4
            B1 = b_ops(h1[:, :hc], h2[:, :hc], h1[:, hc:], h2[:, hc:])
            for k in range(7):
                o = B1[k]
                B2 = b_ops(o[:Q4, :qc], o[Q4:, :qc], o[:Q4, qc:], o[Q4:, qc:])
                for t in range(7):
                    m = dot_nt(wd[jd, 7 * k + t], B2[t].astype(bf16))
                    i = 7 * k + t
                    accs[i] = m if accs[i] is None else accs[i] + m

        prev = stage1(0)
        hs = []
        for j in range(NCH):
            nxt = stage1(j + 1) if j + 1 < NCH else None
            hs.append(stage2(prev))
            if len(hs) == 2:
                stage3(j // 2, hs)
                hs = []
            prev = nxt
        Ms = [cat4(*c_comb(accs[7 * k:7 * k + 7])) for k in range(7)]
        accT = cat4(*c_comb(Ms))
        xnew = x + accT
        xs[:, r] = xnew
        ostage[:, r] = xnew.astype(bf16)

        @pl.when(layer == 1)
        def _():
            pltpu.make_async_copy(ostage.at[:, r], o_hbm.at[:, r], osems.at[b]).start()

    def layer_body(layer, _):
        attn_phase()

        @pl.when(layer == 0)
        def _():
            prep_ffn()

        def fb(b, _):
            ffn_block(b, layer)
            return 0
        lax.fori_loop(0, NB, fb, 0)
        return 0
    lax.fori_loop(0, 2, layer_body, 0)
    for b in range(NB):
        pltpu.make_async_copy(ostage.at[:, b * M:(b + 1) * M], o_hbm.at[:, b * M:(b + 1) * M], osems.at[b]).wait()


def call(x2, wqkv, wo, wg, wu, wd_):
    hbm = pl.BlockSpec(memory_space=pltpu.HBM)
    return pl.pallas_call(
        kernel,
        out_shape=jax.ShapeDtypeStruct((D, S), bf16),
        in_specs=[hbm] * 6,
        out_specs=hbm,
        scratch_shapes=[
            pltpu.VMEM((D, S), bf16),
            pltpu.VMEM((D, S), f32),
            pltpu.VMEM((D, 3 * D), bf16),
            pltpu.VMEM((D, D), bf16),
            pltpu.VMEM((D, F), bf16),
            pltpu.VMEM((D, F), bf16),
            pltpu.VMEM((D, F), bf16),
            pltpu.VMEM((3 * D, 128), f32),
            pltpu.VMEM((3 * D, 640), bf16),
            pltpu.VMEM((D, 640), bf16),
            pltpu.VMEM((NCH, 49, 128, 128), bf16),
            pltpu.VMEM((NCH, 2, 64, CF), bf16),
            pltpu.VMEM((NDC, 49, 144, 128), bf16),
            pltpu.VMEM((D, S), bf16),
            pltpu.SemaphoreType.DMA((6,)),
            pltpu.SemaphoreType.DMA((NB,)),
        ],
        compiler_params=pltpu.CompilerParams(vmem_limit_bytes=120 * 1024 * 1024),
    )(x2, wqkv, wo, wg, wu, wd_)


@jax.jit
def pallas_interleave_layers__sliding_local_dilated__glu_gated_geglu__prompt_kernel(
    A_x, A_wqkv, A_wo, B_x, B_w_gate, B_w_up, B_w_down,
):
    out = call(A_x.reshape(S, D).T, A_wqkv, A_wo, B_w_gate, B_w_up, B_w_down.T)
    return out.T.reshape(1, S, D)
```

```python
import functools
import jax
import jax.numpy as jnp
from jax import lax
import jax.experimental.pallas as pl
import jax.experimental.pallas.tpu as pltpu

S, D, F = 2048, 576, 4608
NH, DH, WIN, DIL = 32, 18, 8, 2
M = 512
H2, Q4 = M // 2, M // 4
NB = S // M
CF = 256
NCH = F // CF
DCH = 512
NDC = F // DCH
TC = S // 2
C0 = 0.7978845608028654
C1 = 0.044715 * C0
f32 = jnp.float32
bf16 = jnp.bfloat16
JB = 3
NT = 3
TP = 48
HPOS = 1
CPOS = 5
TPOS = 3
DEFER = True
QKV_L = 0
WO_L = 0
HG = 8
TG = 4
NPIECE = 4
SKIP_FFN = False
SKIP_LAYERS = False
SKIP_WPREP = False
SKIP_INPERM = False
SKIP_OUTPERM = False
NO_FFN_DMA = False


def dot(a, b):
    return jnp.dot(a, b, preferred_element_type=f32)


def dot_nt(a, b):
    return lax.dot_general(a, b, (((1,), (1,)), ((), ())), preferred_element_type=f32)


def a_ops(A11, A12, A21, A22):
    return [(A11 + A22), (A21 + A22), A11, A22, (A11 + A12), (A21 - A11), (A12 - A22)]


def b_ops(B11, B12, B21, B22):
    return [B11 + B22, B11, B12 - B22, B21 - B11, B22, B11 + B12, B21 + B22]


def c_comb(Ms):
    C11 = Ms[0] + Ms[3] - Ms[4] + Ms[6]
    C12 = Ms[2] + Ms[4]
    C21 = Ms[1] + Ms[3]
    C22 = Ms[0] - Ms[1] + Ms[2] + Ms[5]
    return C11, C12, C21, C22


def cat4(C11, C12, C21, C22):
    return jnp.concatenate([jnp.concatenate([C11, C12], axis=1),
                            jnp.concatenate([C21, C22], axis=1)], axis=0)


def quad(X):
    r, c = X.shape[0] // 2, X.shape[1] // 2
    return X[:r, :c], X[:r, c:], X[r:, :c], X[r:, c:]


def a_ops2(X):
    out = []
    for o in a_ops(*quad(X)):
        out += a_ops(*quad(o))
    return out


def b_ops2(X):
    out = []
    for o in b_ops(*quad(X)):
        out += b_ops(*quad(o))
    return out


def c_comb2(Ms):
    return cat4(*c_comb([cat4(*c_comb(Ms[7 * k:7 * k + 7])) for k in range(7)]))


def layernorm_t(x):
    m = jnp.mean(x, axis=0, keepdims=True)
    d = x - m
    v = jnp.mean(d * d, axis=0, keepdims=True)
    return d * lax.rsqrt(v + 1e-5)


def kernel(x_hbm, wqkv_hbm, wo_hbm, wg_hbm, wu_hbm, wd_hbm, o_hbm,
           xin, xs, wqkv_raw, wo_raw, wg_raw, wu_raw, wd_raw,
           tmpT, wq_ops, wq_left, wo_ops, wo_left, wa, wl, wd,
           qkv0, qkv1, rot0, rot1, o0, o1, ops_s, xl_s, acc_s, ostage, sems, wsems, osem):
    cp_x = pltpu.make_async_copy(x_hbm, xin, sems.at[0])
    cp_qkv = pltpu.make_async_copy(wqkv_hbm, wqkv_raw, sems.at[1])
    cp_wo = pltpu.make_async_copy(wo_hbm, wo_raw, sems.at[2])
    cp_x.start(); cp_qkv.start(); cp_wo.start()

    def wcopies0(jd):
        c = slice(jd * DCH, (jd + 1) * DCH)
        return [pltpu.make_async_copy(wg_hbm.at[:, c], wg_raw.at[:, c], wsems.at[0, jd]),
                pltpu.make_async_copy(wu_hbm.at[:, c], wu_raw.at[:, c], wsems.at[1, jd]),
                pltpu.make_async_copy(wd_hbm.at[:, c], wd_raw.at[:, c], wsems.at[2, jd])]

    cp_x.wait()
    for jd in range(NDC):
        for cp in wcopies0(jd):
            cp.start()
    for kg in range(0 if SKIP_INPERM else 5):
        kw = 128 if kg < 4 else 64
        blk = xin[kg * 128:kg * 128 + kw, :].astype(f32)
        if kw < 128:
            blk = jnp.concatenate([blk, jnp.zeros((128 - kw, S), f32)], axis=0)
        tmpT[kg] = blk.T
    if SKIP_INPERM:
        xs[...] = xin[...].astype(f32)
    for kg in range(0 if SKIP_INPERM else 5):
        kw = 128 if kg < 4 else 64
        for c in range(16):
            t = 2 * (c % 8) + c // 8
            tile = tmpT[kg, pl.ds(t, 128, stride=16), :]
            xs[kg * 128:kg * 128 + kw, c * 128:(c + 1) * 128] = tile.T[0:kw, :]

    cp_qkv.wait()
    for kg in range(0 if SKIP_WPREP else 5):
        kw = 128 if kg < 4 else 64
        blk = wqkv_raw[kg * 128:kg * 128 + kw, :].astype(f32)
        if kw < 128:
            blk = jnp.concatenate([blk, jnp.zeros((128 - kw, 3 * D), f32)], axis=0)
        tmpT[kg, 0:3 * D, :] = blk.T

    def wq_piece(kg, m):
        p, rem = divmod(m, 36)
        d, hh = divmod(rem, 2)
        return tmpT[kg, pl.ds(p * D + 16 * hh * DH + d, 16, stride=DH), :]

    if SKIP_WPREP:
        wq_ops[...] = jnp.zeros(wq_ops.shape, bf16)
    elif QKV_L == 2:
        for m in range(27):
            X = [[wq_piece(kq, nq * 27 + m) for kq in range(4)] for nq in range(4)]
            def blk2(nh, kh):
                return [[X[2 * nh + a][2 * kh + b] for b in range(2)] for a in range(2)]
            L1 = a_ops_struct([blk2(0, 0), blk2(0, 1), blk2(1, 0), blk2(1, 1)])
            for k in range(7):
                o = L1[k]
                L2 = a_ops(o[0][0], o[0][1], o[1][0], o[1][1])
                for t in range(7):
                    wq_ops[7 * k + t, m * 16:(m + 1) * 16, :] = L2[t].astype(bf16)
    elif QKV_L == 1:
        for m in range(54):
            X = [[wq_piece(kq, nh * 54 + m) for kq in range(4)] for nh in range(2)]
            P = lambda nh, kh: jnp.concatenate([X[nh][2 * kh], X[nh][2 * kh + 1]], axis=1)
            for k, t in enumerate(a_ops(P(0, 0), P(0, 1), P(1, 0), P(1, 1))):
                wq_ops[k, m * 16:(m + 1) * 16, :] = t.astype(bf16)
    else:
        for kg in range(5):
            for m in range(108):
                wq_ops[m * 16:(m + 1) * 16, kg * 128:(kg + 1) * 128] = wq_piece(kg, m).astype(bf16)
    if QKV_L > 0:
        for m in range(108):
            wq_left[m * 16:(m + 1) * 16, :] = wq_piece(4, m).astype(bf16)

    cp_wo.wait()
    for ng in range(0 if SKIP_WPREP else 5):
        nw = 128 if ng < 4 else 64
        blk = wo_raw[:, ng * 128:ng * 128 + nw].astype(f32)
        if nw < 128:
            blk = jnp.concatenate([blk, jnp.zeros((D, 128 - nw), f32)], axis=1)
        tmpT[0, 0:D, :] = blk
        perm = jnp.concatenate([tmpT[0, pl.ds(d, NH, stride=DH), :] for d in range(DH)], axis=0)
        perm = jnp.concatenate([perm, jnp.zeros((64, 128), f32)], axis=0)
        pt = perm.T
        for kq in range(5):
            tmpT[1 + kq % 4, 1024 * (kq // 4) + ng * 128:1024 * (kq // 4) + (ng + 1) * 128, :] = pt[:, kq * 128:(kq + 1) * 128]
    woT = [tmpT[1 + kq, 0:D, :] for kq in range(4)]
    wo_left[...] = jnp.zeros(wo_left.shape, bf16)
    if SKIP_WPREP:
        wo_ops[...] = jnp.zeros(wo_ops.shape, bf16)
    elif WO_L == 2:
        Xo = jnp.concatenate(woT, axis=1)
        for i, t in enumerate(a_ops2(Xo)):
            wo_ops[i] = t.astype(bf16)
    else:
        for kq in range(4):
            wo_ops[:, kq * 128:(kq + 1) * 128] = woT[kq].astype(bf16)
        wo_ops[:, 512:640] = tmpT[1, 1024:1024 + D, :].astype(bf16)

    lane = lax.broadcasted_iota(jnp.int32, (HG, 128), 1)

    def put_qkv(dst, rot, r0, c0, val):
        nr, nc = val.shape
        dst[r0:r0 + nr, c0:c0 + nc] = val
        lo = max(r0, D)
        if lo < r0 + nr:
            for cc in range(c0 // 128, (c0 + nc) // 128):
                if cc >= 1:
                    t = val[lo - r0:, cc * 128 - c0:(cc + 1) * 128 - c0]
                    rot[lo - D:r0 + nr - D, (cc - 1) * 128:cc * 128] = pltpu.roll(t, 1, 1)

    def qkv_proj(p, dst, rot):
        xn = layernorm_t(xs[:, p * TC:(p + 1) * TC])
        xl = jnp.concatenate([xn[512:576], xn[512:576]], axis=0).astype(bf16)
        if QKV_L == 2:
            for hb in range(2):
                xb = xn[:, hb * 512:(hb + 1) * 512]
                Bo = [t.astype(bf16) for t in b_ops2(xb[0:512])]
                xlb = xl[:, hb * 512:(hb + 1) * 512]
                for rc in range(3):
                    Ms = [dot(wq_ops[i, rc * 144:(rc + 1) * 144, :], Bo[i]) for i in range(49)]
                    C = c_comb2(Ms)
                    for nq in range(4):
                        r0 = nq * 432 + rc * 144
                        left = dot(wq_left[r0:r0 + 144, :], xlb)
                        put_qkv(dst, rot, r0, hb * 512, C[nq * 144:(nq + 1) * 144] + left)
                    yield
        elif QKV_L == 1:
            B1 = b_ops(*quad(xn[0:512]))
            Mk = []
            for k in range(7):
                Mk.append(dot(wq_ops[k], B1[k].astype(bf16)))
                yield
            C = c_comb(Mk)
            for i, (rr, cc) in enumerate([(0, 0), (0, 1), (1, 0), (1, 1)]):
                left = dot(wq_left[rr * 864:(rr + 1) * 864, :], xl[:, cc * 512:(cc + 1) * 512])
                put_qkv(dst, rot, rr * 864, cc * 512, C[i] + left)
            yield
        else:
            xb = jnp.concatenate([xn, xn[512:576]], axis=0).astype(bf16)
            for rr in range(NPIECE):
                rows = slice(rr * (1728 // NPIECE), (rr + 1) * (1728 // NPIECE))
                put_qkv(dst, rot, rr * (1728 // NPIECE), 0, dot(wq_ops[rows, :], xb))
                yield

    scale = DH ** -0.5

    def attn_vpu(src, rsrc, dst, rlist):
        for r0 in rlist:
            for hg in range(NH // HG):
                def shifted(base, d):
                    row = base + d * NH + hg * HG
                    tiles = {}
                    rot = {}
                    def get(rr):
                        if rr >= 0:
                            if rr not in tiles:
                                tiles[rr] = src[row:row + HG, rr * 128:(rr + 1) * 128]
                            return tiles[rr]
                        if rr not in rot:
                            rot[rr] = rsrc[row - D:row - D + HG, (rr + 7) * 128:(rr + 8) * 128]
                        return rot[rr]
                    return [[get(r - w) for r in range(r0, r0 + TG)] for w in range(WIN)]
                logits = [[None] * TG for _ in range(WIN)]
                for d in range(DH):
                    row = d * NH + hg * HG
                    q = [src[row:row + HG, r * 128:(r + 1) * 128] for r in range(r0, r0 + TG)]
                    ks = shifted(D, d)
                    for w in range(WIN):
                        for i in range(TG):
                            pr = q[i] * ks[w][i]
                            logits[w][i] = pr if logits[w][i] is None else logits[w][i] + pr
                ps = [[None] * TG for _ in range(WIN)]
                for i in range(TG):
                    r = r0 + i
                    ls = []
                    for w in range(WIN):
                        l = logits[w][i] * scale
                        if r < w:
                            l = jnp.where(lane >= 1, l, -1e9)
                        ls.append(l)
                    mx = ls[0]
                    for w in range(1, WIN):
                        mx = jnp.maximum(mx, ls[w])
                    es = [jnp.exp(l - mx) for l in ls]
                    ssum = es[0]
                    for w in range(1, WIN):
                        ssum = ssum + es[w]
                    inv = 1.0 / ssum
                    for w in range(WIN):
                        ps[w][i] = es[w] * inv
                for d in range(DH):
                    row = d * NH + hg * HG
                    vs = shifted(2 * D, d)
                    for i in range(TG):
                        r = r0 + i
                        o = None
                        for w in range(WIN):
                            pr = ps[w][i] * vs[w][i]
                            o = pr if o is None else o + pr
                        dst[row:row + HG, r * 128:(r + 1) * 128] = o
                yield

    def wo_proj(p, src, cols):
        if WO_L == 2:
            for cc in cols:
                c0 = cc[0] * 128
                o = src[:, c0:c0 + 512]
                Bo = [t.astype(bf16) for t in b_ops2(o[0:512])]
                ol = jnp.concatenate([o[512:576], o[512:576]], axis=0).astype(bf16)
                Ms = [dot(wo_ops[i], Bo[i]) for i in range(49)]
                xs[:, p * TC + c0:p * TC + c0 + 512] += c_comb2(Ms) + dot(wo_left[...], ol)
                yield
        else:
            for cc in cols:
                W = 128 * len(cc)
                c0 = cc[0] * 128
                o = src[:, c0:c0 + W]
                ob = jnp.concatenate([o, o[512:576]], axis=0).astype(bf16)
                xs[:, p * TC + c0:p * TC + c0 + W] += dot(wo_ops[...], ob)
                yield

    def interleave(*gens):
        gens = list(gens)
        while gens:
            for g in list(gens):
                try:
                    next(g)
                except StopIteration:
                    gens.remove(g)

    def attn_phase(prep):
        R = list(range(0, 8, TG))
        h = len(R) // 2
        ex = (lambda jds: [prep_ffn(jds)]) if prep else (lambda jds: [])
        interleave(qkv_proj(0, qkv0, rot0))
        interleave(qkv_proj(1, qkv1, rot1), attn_vpu(qkv0, rot0, o0, R), *ex([0, 1, 2, 3]))
        interleave(wo_proj(0, o0, [(0, 1), (2, 3), (4, 5), (6, 7)]), attn_vpu(qkv1, rot1, o1, R[:h]), *ex([4, 5]))
        interleave(wo_proj(1, o1, [(0, 1), (2, 3)]), attn_vpu(qkv1, rot1, o1, R[h:]), *ex([6, 7]))
        interleave(wo_proj(1, o1, [(4, 5), (6, 7)]), *ex([8]))

    def wcopies(jd):
        c = slice(jd * DCH, (jd + 1) * DCH)
        return [pltpu.make_async_copy(wg_hbm.at[:, c], wg_raw.at[:, c], wsems.at[0, jd]),
                pltpu.make_async_copy(wu_hbm.at[:, c], wu_raw.at[:, c], wsems.at[1, jd]),
                pltpu.make_async_copy(wd_hbm.at[:, c], wd_raw.at[:, c], wsems.at[2, jd])]

    def prep_ffn():
        for jd in range(NDC):
            for cp in wcopies(jd):
                cp.wait()

        def gu_chunk(j, _):
            c = pl.ds(pl.multiple_of(j * CF, CF), CF)
            for r in range(0, 128, 32):
                ld = lambda ref: jnp.concatenate([ref[kq * 128 + r:kq * 128 + r + 32, c] for kq in range(4)], axis=0).astype(f32)
                g = ld(wg_raw); u = ld(wu_raw)
                b1 = b_ops(g[:64], u[:64], g[64:], u[64:])
                for k in range(7):
                    b2 = b_ops(*quad(b1[k]))
                    for t in range(7):
                        wa[j, 7 * k + t, r:r + 32, :] = b2[t].astype(bf16)
            wl[j, 0] = wg_raw[512:576, c]
            wl[j, 1] = wu_raw[512:576, c]
            return 0
        lax.fori_loop(0, NCH, gu_chunk, 0)

        def d_chunk(jd, _):
            c = pl.ds(pl.multiple_of(jd * DCH, DCH), DCH)
            for r in range(0, 144, 48):
                wT = jnp.concatenate([wd_raw[nq * 144 + r:nq * 144 + r + 48, c] for nq in range(4)], axis=0).astype(f32) * 0.5
                for i, t in enumerate(a_ops2(wT)):
                    wd[jd, i, r:r + 48, :] = t.astype(bf16)
            return 0
        lax.fori_loop(0, NDC, d_chunk, 0)

    def ffn_head(b, slot):
        r = pl.ds(pl.multiple_of(b * M, M), M)
        xf = layernorm_t(xs[:, r]).T
        xl_ = xf[:, 512:576].astype(bf16)
        ov = [t.astype(bf16) for t in a_ops2(xf[:, 0:512])]

        def commit():
            xl_s[slot] = xl_
            for i, t in enumerate(ov):
                ops_s[slot, i] = t
        return commit

    def ffn_tail(b):
        r = pl.ds(pl.multiple_of(b * M, M), M)
        xs[:, r] += c_comb2([acc_s[0, i] for i in range(49)])

    def ffn_body(b, t):
        sl = 0
        xl = xl_s[sl]

        def stage1(j):
            Ms = []
            for k in range(7):
                m = [dot(ops_s[sl, 7 * k + u], wa[j, 7 * k + u]) for u in range(7)]
                Ms.append(cat4(*c_comb(m)))
            return Ms, dot(xl, wl[j, 0]), dot(xl, wl[j, 1])

        def act(g, u):
            z = g * (C0 + C1 * (g * g))
            a = g * u
            return a + a * jnp.tanh(z)

        def stage2(res):
            Ms, gl, ul = res
            g1, u1, g2, u2 = c_comb(Ms)
            g1 = g1 + gl[:H2]; u1 = u1 + ul[:H2]; g2 = g2 + gl[H2:]; u2 = u2 + ul[H2:]
            return act(g1, u1), act(g2, u2)

        def hops(hs):
            h1 = jnp.concatenate([h[0] for h in hs], axis=1)
            h2 = jnp.concatenate([h[1] for h in hs], axis=1)
            hc = DCH // 2
            out = []
            for o in b_ops(h1[:, :hc], h2[:, :hc], h1[:, hc:], h2[:, hc:]):
                q1, q2, q3, q4 = quad(o)
                out += [v.astype(bf16) for v in b_ops(q1, q3, q2, q4)]
            return out

        def stage3(jd, B2, firstpair):
            for i in range(49):
                old = acc_s[sl, i]
                if firstpair:
                    old = jnp.where(t == 0, 0.0, old)
                acc_s[sl, i] = old + dot_nt(wd[jd, i], B2[i])

        n = 2 * JB
        j0 = t * n
        prev = stage1(j0)
        hs = []
        pend = None
        for i in range(n):
            nxt = stage1(j0 + i + 1) if i + 1 < n else None
            if pend is not None and (DEFER or nxt is not None):
                stage3(*pend); pend = None
            hs.append(stage2(prev))
            if len(hs) == 2:
                pend = (t * JB + i // 2, hops(hs), i // 2 == 0)
                hs = []
                if not DEFER:
                    stage3(*pend); pend = None
            prev = nxt
        if pend is not None:
            stage3(*pend)

    def ffn_phase():
        ffn_head(0, 0)()

        def blk(b, _):
            def inner(t, _):
                ffn_body(b, t)
                return 0
            lax.fori_loop(0, NT, inner, 0)
            ffn_tail(b)
            ffn_head(jnp.minimum(b + 1, NB - 1), 0)()
            return 0
        lax.fori_loop(0, NB, blk, 0)

    def layer_body(layer, _):
        attn_phase(False)

        @pl.when(layer == 0)
        def _():
            prep_ffn()
        ffn_phase()
        return 0
    lax.fori_loop(0, 2, layer_body, 0)

    for kg in range(5):
        kw = 128 if kg < 4 else 64
        for c in range(16):
            t = 2 * (c % 8) + c // 8
            tile = xs[kg * 128:kg * 128 + kw, c * 128:(c + 1) * 128]
            if kw < 128:
                tile = jnp.concatenate([tile, jnp.zeros((128 - kw, 128), f32)], axis=0)
            tmpT[kg, pl.ds(t, 128, stride=16), :] = tile.T
        ostage[kg * 128:kg * 128 + kw, :] = tmpT[kg].T[0:kw, :].astype(bf16)
        pltpu.make_async_copy(ostage.at[kg * 128:kg * 128 + kw, :], o_hbm.at[kg * 128:kg * 128 + kw, :], osem.at[kg]).start()
    for kg in range(5):
        kw = 128 if kg < 4 else 64
        pltpu.make_async_copy(ostage.at[kg * 128:kg * 128 + kw, :], o_hbm.at[kg * 128:kg * 128 + kw, :], osem.at[kg]).wait()


def a_ops_struct(Q):
    A11, A12, A21, A22 = Q
    def add(X, Y):
        return [[X[a][b] + Y[a][b] for b in range(2)] for a in range(2)]
    def sub(X, Y):
        return [[X[a][b] - Y[a][b] for b in range(2)] for a in range(2)]
    return [add(A11, A22), add(A21, A22), A11, A22, add(A11, A12), sub(A21, A11), sub(A12, A22)]


def call(x2, wqkv, wo, wg, wu, wd_):
    hbm = pl.BlockSpec(memory_space=pltpu.HBM)
    return pl.pallas_call(
        kernel,
        out_shape=jax.ShapeDtypeStruct((D, S), bf16),
        in_specs=[hbm] * 6,
        out_specs=hbm,
        scratch_shapes=[
            pltpu.VMEM((D, S), bf16),
            pltpu.VMEM((D, S), f32),
            pltpu.VMEM((D, 3 * D), bf16),
            pltpu.VMEM((D, D), bf16),
            pltpu.VMEM((D, F), bf16),
            pltpu.VMEM((D, F), bf16),
            pltpu.VMEM((D, F), bf16),
            pltpu.VMEM((5, S, 128), f32),
            pltpu.VMEM({2: (49, 432, 128), 1: (7, 864, 256), 0: (3 * D, 640)}[QKV_L], bf16),
            pltpu.VMEM((3 * D, 128), bf16),
            pltpu.VMEM((49, 144, 128) if WO_L == 2 else (D, 640), bf16),
            pltpu.VMEM((D, 128), bf16),
            pltpu.VMEM((NCH, 49, 128, 128), bf16),
            pltpu.VMEM((NCH, 2, 64, CF), bf16),
            pltpu.VMEM((NDC, 49, 144, 128), bf16),
            pltpu.VMEM((3 * D, TC), f32),
            pltpu.VMEM((3 * D, TC), f32),
            pltpu.VMEM((2 * D, 7 * 128), f32),
            pltpu.VMEM((2 * D, 7 * 128), f32),
            pltpu.VMEM((D, TC), f32),
            pltpu.VMEM((D, TC), f32),
            pltpu.VMEM((1, 49, 128, 128), bf16),
            pltpu.VMEM((1, M, 64), bf16),
            pltpu.VMEM((1, 49, 144, 128), f32),
            pltpu.VMEM((D, S), bf16),
            pltpu.SemaphoreType.DMA((3,)),
            pltpu.SemaphoreType.DMA((3, NDC)),
            pltpu.SemaphoreType.DMA((5,)),
        ],
        compiler_params=pltpu.CompilerParams(vmem_limit_bytes=126 * 1024 * 1024),
    )(x2, wqkv, wo, wg, wu, wd_)


@jax.jit
def pallas_interleave_layers__sliding_local_dilated__glu_gated_geglu__prompt_kernel(
    A_x, A_wqkv, A_wo, B_x, B_w_gate, B_w_up, B_w_down,
):
    out = call(A_x.reshape(S, D).T, A_wqkv, A_wo, B_w_gate, B_w_up, B_w_down.T)
    return out.T.reshape(1, S, D)
```
